```python
import jax
import jax.numpy as jnp

def _softmax(x, axis=-1):
    return jax.nn.softmax(x, axis=axis)
def _gelu(x):
    return jax.nn.gelu(x, approximate=True)
def _silu(x):
    return jax.nn.silu(x)
def _sigmoid(x):
    return jax.nn.sigmoid(x)
def _layernorm(x, axis=-1, eps=1e-5):
    m = jnp.mean(x, axis=axis, keepdims=True)
    v = jnp.var(x, axis=axis, keepdims=True)
    return (x - m) / jnp.sqrt(v + eps)
def _scatter_add(tgt, idx, src, axis=0):
    return tgt.at[idx].add(src)
def _segment_sum(src, seg, n):
    return jax.ops.segment_sum(src, seg, n)
class _Rng:
    def __init__(self, key):
        self._k = key
    def _next(self):
        self._k, sub = jax.random.split(self._k)
        return sub
    def normal(self, shape):
        return jax.random.normal(self._next(), shape, dtype=jnp.bfloat16)
    def randint(self, lo, hi, shape):
        return jax.random.randint(self._next(), shape, lo, hi, dtype=jnp.int32)
    def uniform(self, shape, lo=0.0, hi=1.0):
        return jax.random.uniform(self._next(), shape, jnp.bfloat16, lo, hi)
    def permutation(self, n):
        return jax.random.permutation(self._next(), n)


kernel_name = 'sequential_preLN__compressed_kv_cla__moe_arch_mod__prompt'

def setup_inputs():
    _rng = _Rng(jax.random.key(int.from_bytes(__import__("os").urandom(4), "little")))
    _w = (lambda a: (lambda t: t.astype(jnp.bfloat16) if jnp.issubdtype(t.dtype, jnp.floating) else t)(jnp.asarray(a)))
    def _A_setup():
        B, H, Sq, Sk, D, M = 1, 32, 2048, 2048, 128, 1024
        Dc = 4 * D
        return {
            "x": _w((lambda *s: _rng.normal(s) * 0.05)(B, Sq, M)),
            "c_kv": _w((lambda *s: _rng.normal(s) * 0.05)(B, Sk, Dc)),
            "w_q": _w((lambda *s: _rng.normal(s) * 0.05)(M, H, D) * (M ** -0.5)),
            "w_uk": _w((lambda *s: _rng.normal(s) * 0.05)(Dc, H, D) * (Dc ** -0.5)),
            "w_uv": _w((lambda *s: _rng.normal(s) * 0.05)(Dc, H, D) * (Dc ** -0.5)),
            "w_o": _w((lambda *s: _rng.normal(s) * 0.05)(H, D, M) * ((H * D) ** -0.5)),
        }
    _A_in = _A_setup()

    def _B_setup():
        B, S, D, F, C = 1, 2048, 1024, 3584, 2
        return {
            "x": _w((lambda *s: _rng.normal(s) * 0.05)(B, S, D)),
            "w_r": _w((lambda *s: _rng.normal(s) * 0.05)(D)),
            "w_gate": _w((lambda *s: _rng.normal(s) * 0.05)(D, F)),
            "w_up": _w((lambda *s: _rng.normal(s) * 0.05)(D, F)),
            "w_down": _w((lambda *s: _rng.normal(s) * 0.05)(F, D)),
        }
    _B_in = _B_setup()

    return {
        "A_x": _A_in["x"],
        "A_c_kv": _A_in["c_kv"],
        "A_w_q": _A_in["w_q"],
        "A_w_uk": _A_in["w_uk"],
        "A_w_uv": _A_in["w_uv"],
        "A_w_o": _A_in["w_o"],
        "B_x": _B_in["x"],
        "B_w_r": _B_in["w_r"],
        "B_w_gate": _B_in["w_gate"],
        "B_w_up": _B_in["w_up"],
        "B_w_down": _B_in["w_down"],
    }

def reference(A_x, A_c_kv, A_w_q, A_w_uk, A_w_uv, A_w_o, B_x, B_w_r, B_w_gate, B_w_up, B_w_down):
    def _A_ref(x, c_kv, w_q, w_uk, w_uv, w_o):
        B, Sq, M = x.shape[0], x.shape[1], x.shape[2]
        Sk = c_kv.shape[1]
        H, D = w_q.shape[1], w_q.shape[2]
        q = jnp.einsum("bqm,mhd->bhqd", x, w_q)
        k = jnp.einsum("bkc,chd->bhkd", c_kv, w_uk)
        v = jnp.einsum("bkc,chd->bhkd", c_kv, w_uv)
        scores = jnp.einsum("bhqd,bhkd->bhqk", q, k) * (D ** -0.5)
        off = Sk - Sq
        qi = jnp.arange(Sq)[:, None]
        kj = jnp.arange(Sk)[None, :]
        cmask = kj <= (qi + off)
        scores = jnp.where(cmask[None, None], scores, -1e9)
        p = _softmax(scores, axis=-1)
        ctx = jnp.einsum("bhqk,bhkd->bhqd", p, v)
        return jnp.einsum("bhqd,hdm->bqm", ctx, w_o)

    def _B_ref(x, w_r, w_gate, w_up, w_down):
        B, S, D = x.shape
        C = 2
        r = x @ w_r
        idx = jnp.argsort(-r, axis=-1)[:, :C]
        idx_e = jnp.repeat(idx.reshape(B, C, 1), D, axis=2)
        x_sel = jnp.take_along_axis(x, idx_e, axis=1)
        g = _silu(x_sel @ w_gate)
        u = x_sel @ w_up
        y = (g * u) @ w_down
        r_sel = _sigmoid(jnp.take_along_axis(r, idx, axis=1))
        y = y * r_sel.reshape(B, C, 1)
        b_off = (jnp.arange(B) * S).reshape(B, 1)
        flat_idx = (idx + b_off).reshape(B * C)
        zero = (x * 0.0).reshape(B * S, D)
        upd = _scatter_add(zero, flat_idx, y.reshape(B * C, D), axis=0)
        return x + upd.reshape(B, S, D)

    x = A_x
    h = x + _A_ref(_layernorm(x, axis=-1), A_c_kv, A_w_q, A_w_uk, A_w_uv, A_w_o)
    h2 = h + _B_ref(_layernorm(h, axis=-1), B_w_r, B_w_gate, B_w_up, B_w_down)
    return h2
```

```python
import functools
import math

import jax
import jax.numpy as jnp
import jax.experimental.pallas as pl
import jax.experimental.pallas.tpu as pltpu

S, M, H, D, DC, F = 2048, 1024, 32, 128, 512, 3584
BQ = 256
NB = S // BQ
EPS = 1e-5
QSCALE = (D ** -0.5) * math.log2(math.e)
NEG = -1e30
SELROWS = 16

bf16 = jnp.bfloat16
f32 = jnp.float32


def _dot(a, b):
    return jnp.dot(a, b, preferred_element_type=f32)


def _dot_nt(a, b):
    return jax.lax.dot_general(a, b, (((1,), (1,)), ((), ())), preferred_element_type=f32)


def _ln(x):
    mu = jnp.mean(x, axis=-1, keepdims=True)
    xc = x - mu
    var = jnp.mean(xc * xc, axis=-1, keepdims=True)
    return xc * jax.lax.rsqrt(var + EPS)


def _deinterleave(raw, dst, j, rows):
    for m0 in range(0, rows, 256):
        u = raw[pl.ds(m0 * 16 + j, 256, stride=16), :]
        a = pltpu.bitcast(u << 16, f32).astype(bf16)
        b = pltpu.bitcast(u & jnp.int32(-65536), f32).astype(bf16)
        dst[2 * j, pl.ds(m0, 256), :] = a
        dst[2 * j + 1, pl.ds(m0, 256), :] = b


def _kernel(x_hbm, ckv_hbm, wq_hbm, wuk_hbm, wuv_hbm, wo_hbm, wr_ref, wg_hbm, wu_hbm, wd_hbm,
            out_hbm,
            x_v, ckv_v, wq_v, wuk_v, wuv_v, wo_v, k_c, v_c, xn_v, q_s, ctx0, ctx1, acc_v,
            hn_v, out_v, r_v, sems, osems):
    ctx = (ctx0, ctx1)

    def proj(slot, row0, hn, qslot):
        xn = xn_v[slot]
        ckv = ckv_v[pl.ds(row0, BQ), :]
        q = _dot(xn, wq_v[hn]) * QSCALE
        k = _dot(ckv, wuk_v[hn])
        v = _dot(ckv, wuv_v[hn])
        q_s[qslot] = q.astype(bf16)
        k_c[hn, pl.ds(row0, BQ), :] = k.astype(bf16)
        v_c[hn, pl.ds(row0, BQ), :] = v.astype(bf16)

    def attn(i, h):
        L = (i + 1) * BQ
        q = q_s[h % 2]
        s = _dot_nt(q, k_c[h, pl.ds(0, L), :])
        rows = jax.lax.broadcasted_iota(jnp.int32, (BQ, BQ), 0)
        cols = jax.lax.broadcasted_iota(jnp.int32, (BQ, BQ), 1)
        sd = jnp.where(cols <= rows, s[:, L - BQ:], NEG)
        if i > 0:
            s = jnp.concatenate([s[:, :L - BQ], sd], axis=1)
        else:
            s = sd
        m = jnp.max(s, axis=-1, keepdims=True)
        p = jnp.exp2(s - m)
        l = jnp.sum(p, axis=-1, keepdims=True)
        o = _dot(p.astype(bf16), v_c[h, pl.ds(0, L), :])
        ctx[i % 2][h] = (o / l).astype(bf16)

    def outproj_unit(i, u):
        n = u // 4
        kq = u % 4
        c = ctx[i % 2]
        lhs = jnp.concatenate([c[kq * 8 + t] for t in range(8)], axis=1)
        part = _dot(lhs, wo_v[n, pl.ds(pl.multiple_of(kq * 1024, 1024), 1024), :])
        acc_v[u // 4] = jnp.where(kq == 0, part, acc_v[u // 4] + part)

    def out_copy(i):
        return pltpu.make_async_copy(out_v.at[pl.ds(i * BQ, BQ)], out_hbm.at[pl.ds(i * BQ, BQ)],
                                     osems.at[i])

    def epilogue(i):
        rs = pl.ds(i * BQ, BQ)
        a = jnp.concatenate([acc_v[n] for n in range(M // 128)], axis=1)
        hh = x_v[rs, :].astype(f32) + a
        hn = _ln(hh)
        hnb = hn.astype(bf16)
        hn_v[rs, :] = hnb
        out_v[rs, :] = (hh + hn).astype(bf16)
        r = jnp.sum(hnb.astype(f32) * wr_ref[...].astype(f32), axis=-1, keepdims=True)
        lane = jax.lax.broadcasted_iota(jnp.int32, (8, 128), 1)
        racc = r_v[i // 4]
        for t in range(BQ // 8):
            racc = jnp.where(lane == (i % 4) * 32 + t, r[t * 8:(t + 1) * 8, :], racc)
        r_v[i // 4] = racc
        out_copy(i).start()

    cp_x = pltpu.make_async_copy(x_hbm, x_v, sems.at[0])
    cp_ckv = pltpu.make_async_copy(ckv_hbm, ckv_v, sems.at[1])
    cp_wo = [pltpu.make_async_copy(wo_hbm.at[:, pl.ds(n * 128, 128)], wo_v.at[n], sems.at[2 + n])
             for n in range(8)]

    def phase0(wq_raw, wuk_raw, wuv_raw):
        cq = pltpu.make_async_copy(wq_hbm, wq_raw.bitcast(bf16), sems.at[10])
        ck = pltpu.make_async_copy(wuk_hbm, wuk_raw.bitcast(bf16), sems.at[11])
        cv = pltpu.make_async_copy(wuv_hbm, wuv_raw.bitcast(bf16), sems.at[12])
        cp_x.start()
        cq.start()
        cp_ckv.start()
        ck.start()
        cv.start()
        for c in cp_wo:
            c.start()
        cp_x.wait()
        xn_v[0] = _ln(x_v[pl.ds(0, BQ), :].astype(f32)).astype(bf16)
        r_v[...] = jnp.zeros(r_v.shape, f32)
        cq.wait()

        @pl.loop(0, H // 2)
        def _(j):
            _deinterleave(wq_raw, wq_v, j, M)

        ck.wait()
        cv.wait()

        @pl.loop(0, H // 2)
        def _(j):
            _deinterleave(wuk_raw, wuk_v, j, DC)
            _deinterleave(wuv_raw, wuv_v, j, DC)

        cp_ckv.wait()

    pl.run_scoped(phase0,
                  pltpu.VMEM((M * H // 2, D), jnp.int32),
                  pltpu.VMEM((DC * H // 2, D), jnp.int32),
                  pltpu.VMEM((DC * H // 2, D), jnp.int32))

    def main(wg_v, wu_v, wd_v):
        cg = pltpu.make_async_copy(wg_hbm, wg_v, sems.at[13])
        cu = pltpu.make_async_copy(wu_hbm, wu_v, sems.at[14])
        cd = pltpu.make_async_copy(wd_hbm, wd_v, sems.at[15])
        cg.start()
        cu.start()
        cd.start()

        proj(0, 0, 0, 0)
        for i in range(NB):
            if i + 1 < NB:
                xn_v[(i + 1) % 2] = _ln(x_v[pl.ds((i + 1) * BQ, BQ), :].astype(f32)).astype(bf16)
            if i == 1:
                for c in cp_wo:
                    c.wait()

            def body(h, carry, i=i):
                attn(i, h)
                if i > 0:
                    outproj_unit(i - 1, h)
                nb = jnp.minimum(i + (h == H - 1).astype(jnp.int32), NB - 1)
                proj(nb % 2, pl.multiple_of(nb * BQ, BQ), (h + 1) % H, (h + 1) % 2)
                return carry

            jax.lax.fori_loop(0, H, body, 0)
            if i > 0:
                epilogue(i - 1)

        @pl.loop(0, H)
        def _(u):
            outproj_unit(NB - 1, u)

        epilogue(NB - 1)

        r = r_v[...]
        sub = jax.lax.broadcasted_iota(jnp.int32, r.shape, 1)
        lane = jax.lax.broadcasted_iota(jnp.int32, r.shape, 2)
        half = jax.lax.broadcasted_iota(jnp.int32, r.shape, 0)
        tok = half * 1024 + lane * 8 + sub
        big = jnp.int32(1 << 20)

        def allmax(v):
            return jnp.max(jnp.max(jnp.max(v, axis=0), axis=1, keepdims=True), axis=0, keepdims=True)

        def allmin(v):
            return jnp.min(jnp.min(jnp.min(v, axis=0), axis=1, keepdims=True), axis=0, keepdims=True)

        m1 = allmax(r)
        t1 = allmin(jnp.where(r == m1[None], tok, big))
        r2 = jnp.where(tok == t1[None], -jnp.inf, r)
        m2 = allmax(r2)
        t2 = allmin(jnp.where(r2 == m2[None], tok, big))
        t1s = t1[0, 0]
        t2s = t2[0, 0]

        row = jax.lax.broadcasted_iota(jnp.int32, (SELROWS, M), 0)

        def pick(t):
            base = pl.multiple_of((t // SELROWS) * SELROWS, SELROWS)
            blk = hn_v[pl.ds(base, SELROWS), :].astype(f32)
            return jnp.sum(jnp.where(row == t % SELROWS, blk, 0.0), axis=0, keepdims=True)

        xs = jnp.where(row == 0, pick(t1s), jnp.where(row == 1, pick(t2s), 0.0)).astype(bf16)
        cg.wait()
        cu.wait()
        g = _dot(xs, wg_v[...])
        u = _dot(xs, wu_v[...])
        a = (g * jax.nn.sigmoid(g) * u).astype(bf16)
        cd.wait()
        y = _dot(a, wd_v[...])
        gate = jnp.where(row == 0, jax.nn.sigmoid(m1), jax.nn.sigmoid(m2))
        y = y * gate

        for i in range(NB):
            out_copy(i).wait()

        def fix(t, k):
            base = pl.multiple_of((t // SELROWS) * SELROWS, SELROWS)
            yk = y[k:k + 1, :]
            cur = out_v[pl.ds(base, SELROWS), :].astype(f32)
            out_v[pl.ds(base, SELROWS), :] = jnp.where(row == t % SELROWS, cur + yk, cur).astype(bf16)
            c = pltpu.make_async_copy(out_v.at[pl.ds(base, SELROWS)],
                                      out_hbm.at[pl.ds(base, SELROWS)], osems.at[k])
            c.start()
            c.wait()

        fix(t1s, 0)
        fix(t2s, 1)

    pl.run_scoped(main,
                  pltpu.VMEM((M, F), bf16),
                  pltpu.VMEM((M, F), bf16),
                  pltpu.VMEM((F, M), bf16))


@jax.jit
def pallas_sequential_preLN__compressed_kv_cla__moe_arch_mod__prompt_kernel(
    A_x: jax.Array,
    A_c_kv: jax.Array,
    A_w_q: jax.Array,
    A_w_uk: jax.Array,
    A_w_uv: jax.Array,
    A_w_o: jax.Array,
    B_x: jax.Array,
    B_w_r: jax.Array,
    B_w_gate: jax.Array,
    B_w_up: jax.Array,
    B_w_down: jax.Array,
):
    del B_x
    any_spec = pl.BlockSpec(memory_space=pl.ANY)
    vmem_spec = pl.BlockSpec(memory_space=pltpu.VMEM)
    out = pl.pallas_call(
        _kernel,
        out_shape=jax.ShapeDtypeStruct((S, M), bf16),
        in_specs=[any_spec] * 6 + [vmem_spec] + [any_spec] * 3,
        out_specs=any_spec,
        scratch_shapes=[
            pltpu.VMEM((S, M), bf16),
            pltpu.VMEM((S, DC), bf16),
            pltpu.VMEM((H, M, D), bf16),
            pltpu.VMEM((H, DC, D), bf16),
            pltpu.VMEM((H, DC, D), bf16),
            pltpu.VMEM((M // 128, H * D, 128), bf16),
            pltpu.VMEM((H, S, D), bf16),
            pltpu.VMEM((H, S, D), bf16),
            pltpu.VMEM((2, BQ, M), bf16),
            pltpu.VMEM((2, BQ, D), bf16),
            pltpu.VMEM((H, BQ, D), bf16),
            pltpu.VMEM((H, BQ, D), bf16),
            pltpu.VMEM((M // 128, BQ, 128), f32),
            pltpu.VMEM((S, M), bf16),
            pltpu.VMEM((S, M), bf16),
            pltpu.VMEM((2, 8, 128), f32),
            pltpu.SemaphoreType.DMA((16,)),
            pltpu.SemaphoreType.DMA((NB,)),
        ],
        compiler_params=pltpu.CompilerParams(vmem_limit_bytes=120 * 1024 * 1024),
        name="fused_attn_mod",
    )(
        A_x.reshape(S, M),
        A_c_kv.reshape(S, DC),
        A_w_q.reshape(M * H, D),
        A_w_uk.reshape(DC * H, D),
        A_w_uv.reshape(DC * H, D),
        A_w_o.reshape(H * D, M),
        B_w_r.reshape(1, M),
        B_w_gate,
        B_w_up,
        B_w_down,
    )
    return out.reshape(1, S, M)
```

```python
import math

import jax
import jax.numpy as jnp
import jax.experimental.pallas as pl
import jax.experimental.pallas.tpu as pltpu

S, M, H, D, DC, F = 2048, 1024, 32, 128, 512, 3584
BQ = 512
NB = S // BQ
T = 128
NT = BQ // T
RC = 16
HG = 8
EPS = 1e-5
QSCALE = (D ** -0.5) * math.log2(math.e)
NEG = -1e30
SELROWS = 16

bf16 = jnp.bfloat16
f32 = jnp.float32
i32 = jnp.int32


def _dot(a, b):
    return jnp.dot(a, b, preferred_element_type=f32)


def _dot_nt(a, b):
    return jax.lax.dot_general(a, b, (((1,), (1,)), ((), ())), preferred_element_type=f32)


def _b(w):
    return pltpu.bitcast(w, bf16)


def _w(x):
    return pltpu.bitcast(x.astype(bf16), i32)


def _ln(x):
    mu = jnp.mean(x, axis=-1, keepdims=True)
    xc = x - mu
    var = jnp.mean(xc * xc, axis=-1, keepdims=True)
    return xc * jax.lax.rsqrt(var + EPS)


def _tmax(s):
    m = s[:, :128]
    for j in range(1, s.shape[1] // 128):
        m = jnp.maximum(m, s[:, j * 128:(j + 1) * 128])
    return m


def _deinterleave(raw, dst, g, j, rows):
    flat = raw.at[g].reshape(rows * HG, 128)
    hd = 2 * (g * HG + j)
    for m0 in range(0, rows, 256):
        u = flat[pl.ds(m0 * HG + j, 256, stride=HG), :]
        dst[hd, pl.ds(m0 // 2, 128), :] = _w(pltpu.bitcast(u << 16, f32))
        dst[hd + 1, pl.ds(m0 // 2, 128), :] = _w(pltpu.bitcast(u & jnp.int32(-65536), f32))


def _kernel(x_hbm, ckv_hbm, wq_hbm, wuk_hbm, wuv_hbm, wo_hbm, wr_ref, wg_hbm, wu_hbm, wd_hbm,
            out_hbm,
            x_v, ckv_v, wq_v, wuk_v, wuv_v, wo_v, k_c, v_c, xn_v, q_s, ctx0, ctx1, acc_v,
            hn_v, r_v, s_v, p_v, l_v, m_v, mr_v, sems, osems):
    ctx = (ctx0, ctx1)

    def q_proj(i, h):
        q_s[...] = _w(_dot(_b(xn_v[i % 2]), _b(wq_v[h])) * QSCALE)

    def kv_proj(i, h):
        rows = pl.ds(i * BQ // 2, BQ // 2)
        k = _w(_dot(_b(ckv_v[rows, :]), _b(wuk_v[h])))
        v = _w(_dot(_b(ckv_v[rows, :]), _b(wuv_v[h])))
        return k, v

    def kv_store(i, h, kv):
        rows = pl.ds(i * BQ // 2, BQ // 2)
        k_c[h, rows, :] = kv[0]
        v_c[h, rows, :] = kv[1]

    def sm_tiles(rows, tiles, first):
        rs = pl.ds(rows, RC)
        m = m_v[rs, :]
        l = None if first else l_v[rs, :]
        for c in tiles:
            cs = pl.ds(c * T, T)
            p = jnp.exp2(s_v[rs, cs] - m)
            p_v[pl.ds(rows // 2, RC // 2), cs] = _w(p)
            l = p if l is None else l + p
        l_v[rs, :] = l

    def sm_chunk(i, c):
        for r0 in range(0, BQ, RC):
            nt = NT if c < i else r0 // T + 1
            sm_tiles(r0, range(c * NT, c * NT + nt), c == 0)

    def qk_chunk(i, h, c):
        q = _b(q_s[...])
        if c < i:
            sc = _dot_nt(q, _b(k_c[h, pl.ds(c * BQ // 2, BQ // 2), :]))
            s_v[:, pl.ds(c * BQ, BQ)] = sc
            mt = _tmax(sc)
            mr_v[...] = mt if c == 0 else jnp.maximum(mr_v[...], mt)
            return
        rows = jax.lax.broadcasted_iota(i32, (T, T), 0)
        cols = jax.lax.broadcasted_iota(i32, (T, T), 1)
        for g in range(NT):
            rs = pl.ds(g * T, T)
            w = (g + 1) * T
            sc = _dot_nt(q[g * T:(g + 1) * T], _b(k_c[h, pl.ds(c * BQ // 2, w // 2), :]))
            dg = jnp.where(cols <= rows, sc[:, w - T:], NEG)
            mt = dg
            if g > 0:
                s_v[rs, pl.ds(c * BQ, w - T)] = sc[:, :w - T]
                mt = jnp.maximum(mt, _tmax(sc[:, :w - T]))
            s_v[rs, pl.ds(c * BQ + w - T, T)] = dg
            if c > 0:
                mt = jnp.maximum(mt, mr_v[rs, :])
            m_v[rs, :] = jnp.broadcast_to(jnp.max(mt, axis=-1, keepdims=True), (T, 128))

    def pv(i, h):
        linv = 1.0 / jnp.sum(l_v[...], axis=-1, keepdims=True)
        off = i * BQ
        o = None
        if i > 0:
            o = _dot(_b(p_v[:, pl.ds(0, off)]), _b(v_c[h, pl.ds(0, off // 2), :]))
        for g in range(NT):
            w = (g + 1) * T
            og = _dot(_b(p_v[pl.ds(g * T // 2, T // 2), pl.ds(off, w)]),
                      _b(v_c[h, pl.ds(off // 2, w // 2), :]))
            if o is not None:
                og = og + o[g * T:(g + 1) * T]
            ctx[i % 2][h, pl.ds(g * T // 2, T // 2), :] = _w(og * linv[g * T:(g + 1) * T])

    def outproj_unit(i, u):
        n = u % 8
        kq = u // 8
        c = ctx[i % 2]
        lhs = jnp.concatenate([_b(c[kq * 8 + t]) for t in range(8)], axis=1)
        k0 = kq * 512 if isinstance(u, int) else pl.multiple_of(kq * 512, 512)
        part = _dot(lhs, _b(wo_v[n, pl.ds(k0, 512), :]))
        acc_v[n] = jnp.where(kq == 0, part, acc_v[n] + part)

    def step(ip, hp, i, h, iq, hq):
        if ip >= 0:
            pv(ip, hp)
        q_proj(iq, hq)
        kv = None
        if i + 1 < NB:
            kv = kv_proj(i + 1, h)
        else:
            outproj_unit(i - 1, h)
        for c in range(i + 1):
            sm_chunk(i, c)
            qk_chunk(iq, hq, c)
        if iq > i:
            qk_chunk(iq, hq, iq)
        if i > 0 and i + 1 < NB:
            outproj_unit(i - 1, h)
        if kv is not None:
            kv_store(i + 1, h, kv)

    def out_copy(i):
        return pltpu.make_async_copy(x_v.at[pl.ds(i * BQ, BQ)], out_hbm.at[pl.ds(i * BQ, BQ)],
                                     osems.at[i])

    def epilogue(i, r0, nr):
        rs = pl.ds(i * BQ + r0, nr)
        a = jnp.concatenate([acc_v[n, pl.ds(r0, nr), :] for n in range(M // 128)], axis=1)
        hh = x_v[rs, :].astype(f32) + a
        hn = _ln(hh)
        hnb = hn.astype(bf16)
        hn_v[rs, :] = hnb
        x_v[rs, :] = (hh + hn).astype(bf16)
        r = jnp.sum(hnb.astype(f32) * wr_ref[...].astype(f32), axis=-1, keepdims=True)
        lane = jax.lax.broadcasted_iota(i32, (8, 128), 1)
        t0 = (i * BQ + r0) // 8
        racc = r_v[t0 // 128]
        for t in range(nr // 8):
            racc = jnp.where(lane == (t0 + t) % 128, r[t * 8:(t + 1) * 8, :], racc)
        r_v[t0 // 128] = racc

    def ln_x(i):
        for r0 in range(0, BQ, 128):
            xn_v[i % 2, pl.ds(r0 // 2, 64), :] = _w(_ln(x_v[pl.ds(i * BQ + r0, 128), :].astype(f32)))

    def rows_copy(src, dst, i, s):
        return pltpu.make_async_copy(src.at[pl.ds(i * BQ, BQ)], dst.at[pl.ds(i * BQ, BQ)], sems.at[s])

    cp_x = [rows_copy(x_hbm, x_v, i, i) for i in range(NB)]
    cp_ckv = [rows_copy(ckv_hbm, ckv_v.bitcast(bf16), i, 4 + i) for i in range(NB)]
    cp_wo = [pltpu.make_async_copy(wo_hbm.at[:, pl.ds(n * 128, 128)], wo_v.bitcast(bf16).at[n],
                                   sems.at[8 + n]) for n in range(8)]

    def phase0(wq_raw, wuk_raw, wuv_raw):
        def grp(src, dst, s):
            return [pltpu.make_async_copy(src.bitcast(i32).at[:, pl.ds(g * HG, HG), :], dst.at[g],
                                          sems.at[s + g]) for g in range(2)]

        cq = grp(wq_hbm, wq_raw, 16)
        ck = grp(wuk_hbm, wuk_raw, 18)
        cv = grp(wuv_hbm, wuv_raw, 20)
        for c in (ck[0], cp_ckv[0], cv[0], ck[1], cv[1], cq[0], cp_x[0], cq[1], cp_ckv[1], cp_x[1],
                  *cp_wo, *cp_ckv[2:], *cp_x[2:]):
            c.start()
        r_v[...] = jnp.zeros(r_v.shape, f32)
        cp_ckv[0].wait()
        for g in range(2):
            with jax.named_scope("w_kv"):
                ck[g].wait()
                cv[g].wait()
                if g == 1:
                    cq[0].wait()

            def pair(j, carry, g=g):
                _deinterleave(wuk_raw, wuk_v, g, j, DC)
                _deinterleave(wuv_raw, wuv_v, g, j, DC)
                for t in range(2):
                    h = 2 * (g * HG + j) + t
                    kv_store(0, h, kv_proj(0, h))
                if g == 1:
                    _deinterleave(wq_raw, wq_v, 0, j, M)
                return carry

            with jax.named_scope("pairs"):
                jax.lax.fori_loop(0, HG, pair, 0)
        cp_x[0].wait()
        ln_x(0)
        q_proj(0, 0)
        qk_chunk(0, 0, 0)
        with jax.named_scope("w_q1"):
            cq[1].wait()
        jax.lax.fori_loop(0, HG, lambda j, c: _deinterleave(wq_raw, wq_v, 1, j, M), None)

    with jax.named_scope("phase0"):
        pl.run_scoped(phase0,
                      pltpu.VMEM((2, M, HG, D), i32),
                      pltpu.VMEM((2, DC, HG, D), i32),
                      pltpu.VMEM((2, DC, HG, D), i32))

    def main(wg_v, wu_v, wd_v):
        cg = pltpu.make_async_copy(wg_hbm, wg_v, sems.at[22])
        cu = pltpu.make_async_copy(wu_hbm, wu_v, sems.at[23])
        cd = pltpu.make_async_copy(wd_hbm, wd_v, sems.at[24])
        cg.start()
        cu.start()
        cd.start()

        for i in range(NB):
            with jax.named_scope("head"):
                if i + 1 < NB:
                    cp_ckv[i + 1].wait()
                    cp_x[i + 1].wait()
                if i == 1:
                    for c in cp_wo:
                        c.wait()
                if i >= 2:
                    epilogue(i - 2, 0, BQ)
                    out_copy(i - 2).start()
                step(i - 1, H - 1, i, 0, i, 1)
                if i + 1 < NB:
                    ln_x(i + 1)

            def body(h, carry, i=i):
                step(i, h - 1, i, h, i, h + 1)
                return carry

            with jax.named_scope(f"loop{i}"):
                jax.lax.fori_loop(1, H - 1, body, 0)
            with jax.named_scope("tail"):
                if i + 1 < NB:
                    step(i, H - 2, i, H - 1, i + 1, 0)
                else:
                    pv(i, H - 2)
                    outproj_unit(i - 1, H - 1)
                    for c in range(NB):
                        sm_chunk(i, c)
                    epilogue(i - 1, 0, BQ)
                    out_copy(i - 1).start()
                    pv(i, H - 1)

        last = NB - 1
        with jax.named_scope("lastout"):
            for r0 in range(0, BQ, 256):
                lhs = jnp.concatenate([_b(ctx[last % 2][t, pl.ds(r0 // 2, 128), :]) for t in range(H)],
                                      axis=1)
                for n in range(8):
                    acc_v[n, pl.ds(r0, 256), :] = _dot(lhs, _b(wo_v[n]))
                epilogue(last, r0, 256)
            out_copy(last).start()

        r = r_v[...]
        sub = jax.lax.broadcasted_iota(i32, r.shape, 1)
        lane = jax.lax.broadcasted_iota(i32, r.shape, 2)
        half = jax.lax.broadcasted_iota(i32, r.shape, 0)
        tok = half * 1024 + lane * 8 + sub
        big = jnp.int32(1 << 20)

        def allmax(v):
            return jnp.max(jnp.max(jnp.max(v, axis=0), axis=1, keepdims=True), axis=0, keepdims=True)

        def allmin(v):
            return jnp.min(jnp.min(jnp.min(v, axis=0), axis=1, keepdims=True), axis=0, keepdims=True)

        m1 = allmax(r)
        t1 = allmin(jnp.where(r == m1[None], tok, big))
        r2 = jnp.where(tok == t1[None], -jnp.inf, r)
        m2 = allmax(r2)
        t2 = allmin(jnp.where(r2 == m2[None], tok, big))
        t1s = t1[0, 0]
        t2s = t2[0, 0]

        row = jax.lax.broadcasted_iota(i32, (SELROWS, M), 0)

        def pick(t):
            base = pl.multiple_of((t // SELROWS) * SELROWS, SELROWS)
            blk = hn_v[pl.ds(base, SELROWS), :].astype(f32)
            return jnp.sum(jnp.where(row == t % SELROWS, blk, 0.0), axis=0, keepdims=True)

        xs = jnp.where(row == 0, pick(t1s), jnp.where(row == 1, pick(t2s), 0.0)).astype(bf16)
        cg.wait()
        cu.wait()
        g = _dot(xs, wg_v[...])
        u = _dot(xs, wu_v[...])
        a = (g * jax.nn.sigmoid(g) * u).astype(bf16)
        cd.wait()
        y = _dot(a, wd_v[...])
        gate = jnp.where(row == 0, jax.nn.sigmoid(m1), jax.nn.sigmoid(m2))
        y = y * gate

        for i in range(NB):
            out_copy(i).wait()

        def fix(t, k):
            base = pl.multiple_of((t // SELROWS) * SELROWS, SELROWS)
            yk = y[k:k + 1, :]
            cur = x_v[pl.ds(base, SELROWS), :].astype(f32)
            x_v[pl.ds(base, SELROWS), :] = jnp.where(row == t % SELROWS, cur + yk, cur).astype(bf16)
            c = pltpu.make_async_copy(x_v.at[pl.ds(base, SELROWS)],
                                      out_hbm.at[pl.ds(base, SELROWS)], osems.at[k])
            c.start()
            c.wait()

        fix(t1s, 0)
        fix(t2s, 1)

    pl.run_scoped(main,
                  pltpu.VMEM((M, F), bf16),
                  pltpu.VMEM((M, F), bf16),
                  pltpu.VMEM((F, M), bf16))


@jax.jit
def pallas_sequential_preLN__compressed_kv_cla__moe_arch_mod__prompt_kernel(
    A_x: jax.Array,
    A_c_kv: jax.Array,
    A_w_q: jax.Array,
    A_w_uk: jax.Array,
    A_w_uv: jax.Array,
    A_w_o: jax.Array,
    B_x: jax.Array,
    B_w_r: jax.Array,
    B_w_gate: jax.Array,
    B_w_up: jax.Array,
    B_w_down: jax.Array,
):
    del B_x
    any_spec = pl.BlockSpec(memory_space=pl.ANY)
    vmem_spec = pl.BlockSpec(memory_space=pltpu.VMEM)
    out = pl.pallas_call(
        _kernel,
        out_shape=jax.ShapeDtypeStruct((S, M), bf16),
        in_specs=[any_spec] * 6 + [vmem_spec] + [any_spec] * 3,
        out_specs=any_spec,
        scratch_shapes=[
            pltpu.VMEM((S, M), bf16),
            pltpu.VMEM((S // 2, DC), i32),
            pltpu.VMEM((H, M // 2, D), i32),
            pltpu.VMEM((H, DC // 2, D), i32),
            pltpu.VMEM((H, DC // 2, D), i32),
            pltpu.VMEM((M // 128, H * D // 2, 128), i32),
            pltpu.VMEM((H, S // 2, D), i32),
            pltpu.VMEM((H, S // 2, D), i32),
            pltpu.VMEM((2, BQ // 2, M), i32),
            pltpu.VMEM((BQ // 2, D), i32),
            pltpu.VMEM((H, BQ // 2, D), i32),
            pltpu.VMEM((H, BQ // 2, D), i32),
            pltpu.VMEM((M // 128, BQ, 128), f32),
            pltpu.VMEM((S, M), bf16),
            pltpu.VMEM((2, 8, 128), f32),
            pltpu.VMEM((BQ, S), f32),
            pltpu.VMEM((BQ // 2, S), i32),
            pltpu.VMEM((BQ, 128), f32),
            pltpu.VMEM((BQ, 128), f32),
            pltpu.VMEM((BQ, 128), f32),
            pltpu.SemaphoreType.DMA((25,)),
            pltpu.SemaphoreType.DMA((NB,)),
        ],
        compiler_params=pltpu.CompilerParams(vmem_limit_bytes=124 * 1024 * 1024),
        name="fused_attn_mod",
    )(
        A_x.reshape(S, M),
        A_c_kv.reshape(S, DC),
        A_w_q,
        A_w_uk,
        A_w_uv,
        A_w_o.reshape(H * D, M),
        B_w_r.reshape(1, M),
        B_w_gate,
        B_w_up,
        B_w_down,
    )
    return out.reshape(1, S, M)
```

```python
import math

import jax
import jax.numpy as jnp
import jax.experimental.pallas as pl
import jax.experimental.pallas.tpu as pltpu

S, M, H, D, DC, F = 2048, 1024, 32, 128, 512, 3584
BQ = 512
NB = S // BQ
T = 128
NT = BQ // T
RC = 16
HG = 8
EPS = 1e-5
QSCALE = (D ** -0.5) * math.log2(math.e)
NEG = -1e30
SELROWS = 16
U = (2, 1, 1, 1)

bf16 = jnp.bfloat16
f32 = jnp.float32
i32 = jnp.int32


def _dot(a, b):
    return jnp.dot(a, b, preferred_element_type=f32)


def _dot_nt(a, b):
    return jax.lax.dot_general(a, b, (((1,), (1,)), ((), ())), preferred_element_type=f32)


def _b(w):
    return pltpu.bitcast(w, bf16)


def _w(x):
    return pltpu.bitcast(x.astype(bf16), i32)


def _ln(x):
    mu = jnp.mean(x, axis=-1, keepdims=True)
    xc = x - mu
    var = jnp.mean(xc * xc, axis=-1, keepdims=True)
    return xc * jax.lax.rsqrt(var + EPS)


def _tmax(s):
    m = s[:, :128]
    for j in range(1, s.shape[1] // 128):
        m = jnp.maximum(m, s[:, j * 128:(j + 1) * 128])
    return m


def _deinterleave(raw, dst, jj, rows):
    flat = raw.reshape(2 * rows * HG, 128)
    base = (jj // HG) * rows * HG + jj % HG
    for m0 in range(0, rows, 256):
        u = flat[pl.ds(base + m0 * HG, 256, stride=HG), :]
        dst[2 * jj, pl.ds(m0, 256), :] = pltpu.bitcast(u << 16, f32).astype(bf16)
        dst[2 * jj + 1, pl.ds(m0, 256), :] = pltpu.bitcast(u & jnp.int32(-65536), f32).astype(bf16)


def _kernel(x_hbm, ckv_hbm, wq_hbm, wuk_hbm, wuv_hbm, wo_hbm, wr_ref, wg_hbm, wu_hbm, wd_hbm,
            out_hbm,
            x_v, ckv_v, wq_v, wuk_v, wuv_v, wo_v, k_c, v_c, xn_v, q_s, ctx0, ctx1, acc_v,
            hn_v, r_v, s_v, p_v, l_v, m_v, mr_v, sems, osems):
    ctx = (ctx0, ctx1)

    def q_proj(i, h):
        q_s[...] = (_dot(_b(xn_v[i % 2]), _b(wq_v.bitcast(i32)[h])) * QSCALE).astype(bf16)

    def _k_proj(i, h):
        x = _dot(_b(ckv_v[pl.ds(i * BQ // 2, BQ // 2), :]), _b(wuk_v.bitcast(i32)[h]))
        return x.astype(bf16)

    def _v_proj(i, h):
        x = _dot(_b(ckv_v[pl.ds(i * BQ // 2, BQ // 2), :]), _b(wuv_v.bitcast(i32)[h]))
        return x.astype(bf16)

    def kv_proj(i, h):
        return _k_proj(i, h), _v_proj(i, h)

    def kv_store(i, h, kv):
        k_c[h, pl.ds(i * BQ, BQ), :] = kv[0]
        v_c[h, pl.ds(i * BQ, BQ), :] = kv[1]

    def sm_tiles(rows, tiles, first):
        rs = pl.ds(rows, RC)
        m = m_v[rs, :]
        l = None if first else l_v[rs, :]
        for c in tiles:
            cs = pl.ds(c * T, T)
            p = jnp.exp2(s_v[rs, cs] - m)
            p_v[pl.ds(rows // 2, RC // 2), cs] = _w(p)
            l = p if l is None else l + p
        l_v[rs, :] = l

    def sm_chunk(i, c):
        for r0 in range(0, BQ, RC):
            nt = NT if c < i else r0 // T + 1
            sm_tiles(r0, range(c * NT, c * NT + nt), c == 0)

    def qk_chunk(i, h, c):
        q = _b(q_s.bitcast(i32)[...])
        if c < i:
            sc = _dot_nt(q, _b(k_c.bitcast(i32)[h, pl.ds(c * BQ // 2, BQ // 2), :]))
            s_v[:, pl.ds(c * BQ, BQ)] = sc
            mt = _tmax(sc)
            mr_v[...] = mt if c == 0 else jnp.maximum(mr_v[...], mt)
            return
        rows = jax.lax.broadcasted_iota(i32, (T, T), 0)
        cols = jax.lax.broadcasted_iota(i32, (T, T), 1)
        for g in range(NT):
            rs = pl.ds(g * T, T)
            w = (g + 1) * T
            sc = _dot_nt(q[g * T:(g + 1) * T], _b(k_c.bitcast(i32)[h, pl.ds(c * BQ // 2, w // 2), :]))
            dg = jnp.where(cols <= rows, sc[:, w - T:], NEG)
            mt = dg
            if g > 0:
                s_v[rs, pl.ds(c * BQ, w - T)] = sc[:, :w - T]
                mt = jnp.maximum(mt, _tmax(sc[:, :w - T]))
            s_v[rs, pl.ds(c * BQ + w - T, T)] = dg
            if c > 0:
                mt = jnp.maximum(mt, mr_v[rs, :])
            m_v[rs, :] = jnp.broadcast_to(jnp.max(mt, axis=-1, keepdims=True), (T, 128))

    def pv(i, h):
        linv = 1.0 / jnp.sum(l_v[...], axis=-1, keepdims=True)
        off = i * BQ
        o = None
        if i > 0:
            o = _dot(_b(p_v[:, pl.ds(0, off)]), _b(v_c.bitcast(i32)[h, pl.ds(0, off // 2), :]))
        for g in range(NT):
            w = (g + 1) * T
            og = _dot(_b(p_v[pl.ds(g * T // 2, T // 2), pl.ds(off, w)]),
                      _b(v_c.bitcast(i32)[h, pl.ds(off // 2, w // 2), :]))
            if o is not None:
                og = og + o[g * T:(g + 1) * T]
            ctx[i % 2][h, pl.ds(g * T, T), :] = (og * linv[g * T:(g + 1) * T]).astype(bf16)

    def outproj_unit(i, u):
        n = u % 8
        kq = u // 8
        c = ctx[i % 2].bitcast(i32)
        lhs = jnp.concatenate([_b(c[kq * 8 + t]) for t in range(8)], axis=1)
        k0 = kq * 512 if isinstance(u, int) else pl.multiple_of(kq * 512, 512)
        part = _dot(lhs, _b(wo_v[n, pl.ds(k0, 512), :]))
        acc_v[n] = jnp.where(kq == 0, part, acc_v[n] + part)

    def step(ip, hp, i, h, iq, hq):
        q_proj(iq, hq)
        if ip >= 0:
            pv(ip, hp)
        mid = 0 < i < NB - 1
        if mid:
            outproj_unit(i - 1, h)
        if i == 0:
            k = _k_proj(i + 1, h)
        for c in range(i + 1):
            sm_chunk(i, c)
            qk_chunk(iq, hq, c)
        if iq > i:
            qk_chunk(iq, hq, iq)
        if i == 0:
            kv = (k, _v_proj(i + 1, h))
        elif mid:
            kv = kv_proj(i + 1, h)
        else:
            outproj_unit(i - 1, h)
        if i + 1 < NB:
            kv_store(i + 1, h, kv)

    def out_copy(i):
        return pltpu.make_async_copy(x_v.at[pl.ds(i * BQ, BQ)], out_hbm.at[pl.ds(i * BQ, BQ)],
                                     osems.at[i])

    def epilogue(i, r0, nr):
        rs = pl.ds(i * BQ + r0, nr)
        a = jnp.concatenate([acc_v[n, pl.ds(r0, nr), :] for n in range(M // 128)], axis=1)
        hh = x_v[rs, :].astype(f32) + a
        hn = _ln(hh)
        hnb = hn.astype(bf16)
        hn_v[rs, :] = hnb
        x_v[rs, :] = (hh + hn).astype(bf16)
        r = jnp.sum(hnb.astype(f32) * wr_ref[...].astype(f32), axis=-1, keepdims=True)
        lane = jax.lax.broadcasted_iota(i32, (8, 128), 1)
        t0 = (i * BQ + r0) // 8
        racc = r_v[t0 // 128]
        for t in range(nr // 8):
            racc = jnp.where(lane == (t0 + t) % 128, r[t * 8:(t + 1) * 8, :], racc)
        r_v[t0 // 128] = racc

    def ln_x(i):
        for r0 in range(0, BQ, 128):
            xn_v[i % 2, pl.ds(r0 // 2, 64), :] = _w(_ln(x_v[pl.ds(i * BQ + r0, 128), :].astype(f32)))

    def rows_copy(src, dst, i, s):
        return pltpu.make_async_copy(src.at[pl.ds(i * BQ, BQ)], dst.at[pl.ds(i * BQ, BQ)], sems.at[s])

    cp_x = [rows_copy(x_hbm, x_v, i, i) for i in range(NB)]
    cp_ckv = [rows_copy(ckv_hbm, ckv_v.bitcast(bf16), i, 4 + i) for i in range(NB)]
    cp_wo = [pltpu.make_async_copy(wo_hbm.at[:, pl.ds(n * 128, 128)], wo_v.bitcast(bf16).at[n],
                                   sems.at[8 + n]) for n in range(8)]

    def phase0(wq_raw, wuk_raw, wuv_raw):
        def grp(src, dst, s, rows):
            return [pltpu.make_async_copy(src.bitcast(i32).at[:, pl.ds(g * HG, HG), :], dst.at[pl.ds(g * rows, rows)],
                                          sems.at[s + g]) for g in range(2)]

        cq = grp(wq_hbm, wq_raw, 16, M)
        ck = grp(wuk_hbm, wuk_raw, 18, DC)
        cv = grp(wuv_hbm, wuv_raw, 20, DC)
        for c in (ck[0], cp_ckv[0], cv[0]):
            c.start()
        r_v[...] = jnp.zeros(r_v.shape, f32)
        with jax.named_scope("w0"):
            ck[0].wait()
        for c in (ck[1], cv[1], cq[0], cp_x[0], cq[1]):
            c.start()
        _deinterleave(wuk_raw, wuk_v, 0, DC)
        cv[0].wait()
        _deinterleave(wuv_raw, wuv_v, 0, DC)
        cp_ckv[0].wait()

        def pair(jj, second):
            nxt = jnp.minimum(jj + 1, H // 2 - 1)
            if second:
                @pl.when(jj == HG + HG // 2)
                def _():
                    cq[1].wait()

                t = jj - HG
                _deinterleave(wq_raw, wq_v, 2 * t, M)
                _deinterleave(wq_raw, wq_v, 2 * t + 1, M)
                r0 = pl.multiple_of(t * 64, 64)
                xn_v[0, pl.ds(pl.multiple_of(t * 32, 32), 32), :] = _w(_ln(x_v[pl.ds(r0, 64), :].astype(f32)))
            else:
                @pl.when(jj == HG - 1)
                def _():
                    ck[1].wait()
                    cv[1].wait()

            kvs = [kv_proj(0, 2 * jj + t) for t in range(2)]
            for t in range(2):
                kv_store(0, 2 * jj + t, kvs[t])
            _deinterleave(wuk_raw, wuk_v, nxt, DC)
            _deinterleave(wuv_raw, wuv_v, nxt, DC)

        with jax.named_scope("pairs"):
            jax.lax.fori_loop(0, HG, lambda j, c: pair(j, False), None)
        with jax.named_scope("w1"):
            cq[0].wait()
            cp_x[0].wait()
        for c in (cp_ckv[1], cp_x[1], *cp_wo, *cp_ckv[2:], *cp_x[2:]):
            c.start()
        with jax.named_scope("pairs2"):
            jax.lax.fori_loop(HG, 2 * HG, lambda j, c: pair(j, True), None)
        q_proj(0, 0)
        qk_chunk(0, 0, 0)

    with jax.named_scope("phase0"):
        pl.run_scoped(phase0,
                      pltpu.VMEM((2 * M, HG, D), i32),
                      pltpu.VMEM((2 * DC, HG, D), i32),
                      pltpu.VMEM((2 * DC, HG, D), i32))

    def main(wg_v, wu_v, wd_v):
        cg = pltpu.make_async_copy(wg_hbm, wg_v.bitcast(bf16), sems.at[22])
        cu = pltpu.make_async_copy(wu_hbm, wu_v.bitcast(bf16), sems.at[23])
        cd = pltpu.make_async_copy(wd_hbm, wd_v.bitcast(bf16), sems.at[24])
        cg.start()
        cu.start()
        cd.start()

        for i in range(NB):
            with jax.named_scope("head"):
                if i + 1 < NB:
                    cp_ckv[i + 1].wait()
                    cp_x[i + 1].wait()
                if i == 1:
                    for c in cp_wo:
                        c.wait()
                if i >= 2:
                    epilogue(i - 2, 0, BQ)
                    out_copy(i - 2).start()
                step(i - 1, H - 1, i, 0, i, 1)
                if i + 1 < NB:
                    ln_x(i + 1)

            def body(t, carry, i=i):
                for u in range(U[i]):
                    h = t * U[i] + u + 1
                    step(i, h - 1, i, h, i, h + 1)
                return carry

            with jax.named_scope(f"loop{i}"):
                jax.lax.fori_loop(0, (H - 2) // U[i], body, 0)
            with jax.named_scope("tail"):
                if i + 1 < NB:
                    step(i, H - 2, i, H - 1, i + 1, 0)
                else:
                    pv(i, H - 2)
                    outproj_unit(i - 1, H - 1)
                    for c in range(NB):
                        sm_chunk(i, c)
                    epilogue(i - 1, 0, BQ)
                    out_copy(i - 1).start()
                    pv(i, H - 1)

        last = NB - 1
        with jax.named_scope("lastout"):
            for r0 in range(0, BQ, 256):
                lhs = jnp.concatenate([_b(ctx[last % 2].bitcast(i32)[t, pl.ds(r0 // 2, 128), :]) for t in range(H)],
                                      axis=1)
                for n in range(8):
                    acc_v[n, pl.ds(r0, 256), :] = _dot(lhs, _b(wo_v[n]))
                epilogue(last, r0, 256)
            out_copy(last).start()

        r = r_v[...]
        sub = jax.lax.broadcasted_iota(i32, r.shape, 1)
        lane = jax.lax.broadcasted_iota(i32, r.shape, 2)
        half = jax.lax.broadcasted_iota(i32, r.shape, 0)
        tok = half * 1024 + lane * 8 + sub
        big = jnp.int32(1 << 20)

        def allmax(v):
            return jnp.max(jnp.max(jnp.max(v, axis=0), axis=1, keepdims=True), axis=0, keepdims=True)

        def allmin(v):
            return jnp.min(jnp.min(jnp.min(v, axis=0), axis=1, keepdims=True), axis=0, keepdims=True)

        m1 = allmax(r)
        t1 = allmin(jnp.where(r == m1[None], tok, big))
        r2 = jnp.where(tok == t1[None], -jnp.inf, r)
        m2 = allmax(r2)
        t2 = allmin(jnp.where(r2 == m2[None], tok, big))
        t1s = t1[0, 0]
        t2s = t2[0, 0]

        row = jax.lax.broadcasted_iota(i32, (SELROWS, M), 0)

        def pick(t):
            base = pl.multiple_of((t // SELROWS) * SELROWS, SELROWS)
            blk = hn_v[pl.ds(base, SELROWS), :].astype(f32)
            return jnp.sum(jnp.where(row == t % SELROWS, blk, 0.0), axis=0, keepdims=True)

        xs = jnp.where(row == 0, pick(t1s), jnp.where(row == 1, pick(t2s), 0.0)).astype(bf16)
        cg.wait()
        cu.wait()
        g = _dot(xs, _b(wg_v[...]))
        u = _dot(xs, _b(wu_v[...]))
        a = (g * jax.nn.sigmoid(g) * u).astype(bf16)
        cd.wait()
        y = _dot(a, _b(wd_v[...]))
        gate = jnp.where(row == 0, jax.nn.sigmoid(m1), jax.nn.sigmoid(m2))
        y = y * gate

        for i in range(NB):
            out_copy(i).wait()

        def fix(t, k):
            base = pl.multiple_of((t // SELROWS) * SELROWS, SELROWS)
            yk = y[k:k + 1, :]
            cur = x_v[pl.ds(base, SELROWS), :].astype(f32)
            x_v[pl.ds(base, SELROWS), :] = jnp.where(row == t % SELROWS, cur + yk, cur).astype(bf16)
            c = pltpu.make_async_copy(x_v.at[pl.ds(base, SELROWS)],
                                      out_hbm.at[pl.ds(base, SELROWS)], osems.at[k])
            c.start()
            c.wait()

        fix(t1s, 0)
        fix(t2s, 1)

    pl.run_scoped(main,
                  pltpu.VMEM((M // 2, F), i32),
                  pltpu.VMEM((M // 2, F), i32),
                  pltpu.VMEM((F // 2, M), i32))


@jax.jit
def pallas_sequential_preLN__compressed_kv_cla__moe_arch_mod__prompt_kernel(
    A_x: jax.Array,
    A_c_kv: jax.Array,
    A_w_q: jax.Array,
    A_w_uk: jax.Array,
    A_w_uv: jax.Array,
    A_w_o: jax.Array,
    B_x: jax.Array,
    B_w_r: jax.Array,
    B_w_gate: jax.Array,
    B_w_up: jax.Array,
    B_w_down: jax.Array,
):
    del B_x
    any_spec = pl.BlockSpec(memory_space=pl.ANY)
    vmem_spec = pl.BlockSpec(memory_space=pltpu.VMEM)
    out = pl.pallas_call(
        _kernel,
        out_shape=jax.ShapeDtypeStruct((S, M), bf16),
        in_specs=[any_spec] * 6 + [vmem_spec] + [any_spec] * 3,
        out_specs=any_spec,
        scratch_shapes=[
            pltpu.VMEM((S, M), bf16),
            pltpu.VMEM((S // 2, DC), i32),
            pltpu.VMEM((H, M, D), bf16),
            pltpu.VMEM((H, DC, D), bf16),
            pltpu.VMEM((H, DC, D), bf16),
            pltpu.VMEM((M // 128, H * D // 2, 128), i32),
            pltpu.VMEM((H, S, D), bf16),
            pltpu.VMEM((H, S, D), bf16),
            pltpu.VMEM((2, BQ // 2, M), i32),
            pltpu.VMEM((BQ, D), bf16),
            pltpu.VMEM((H, BQ, D), bf16),
            pltpu.VMEM((H, BQ, D), bf16),
            pltpu.VMEM((M // 128, BQ, 128), f32),
            pltpu.VMEM((S, M), bf16),
            pltpu.VMEM((2, 8, 128), f32),
            pltpu.VMEM((BQ, S), f32),
            pltpu.VMEM((BQ // 2, S), i32),
            pltpu.VMEM((BQ, 128), f32),
            pltpu.VMEM((BQ, 128), f32),
            pltpu.VMEM((BQ, 128), f32),
            pltpu.SemaphoreType.DMA((25,)),
            pltpu.SemaphoreType.DMA((NB,)),
        ],
        compiler_params=pltpu.CompilerParams(vmem_limit_bytes=124 * 1024 * 1024),
        name="fused_attn_mod",
    )(
        A_x.reshape(S, M),
        A_c_kv.reshape(S, DC),
        A_w_q,
        A_w_uk,
        A_w_uv,
        A_w_o.reshape(H * D, M),
        B_w_r.reshape(1, M),
        B_w_gate,
        B_w_up,
        B_w_down,
    )
    return out.reshape(1, S, M)
```
